```python
import os as _os
_os.environ.setdefault('JAX_PLATFORMS', 'cpu')
import jax
import jax.numpy as jnp

def _softmax(x, axis=-1):
    return jax.nn.softmax(x, axis=axis)

def _gelu(x):
    return jax.nn.gelu(x, approximate=True)

def _silu(x):
    return jax.nn.silu(x)

def _sigmoid(x):
    return jax.nn.sigmoid(x)

def _layernorm(x, axis=-1, eps=1e-05):
    m = jnp.mean(x, axis=axis, keepdims=True)
    v = jnp.var(x, axis=axis, keepdims=True)
    return (x - m) / jnp.sqrt(v + eps)

def _scatter_add(tgt, idx, src, axis=0):
    return tgt.at[idx].add(src)

def _segment_sum(src, seg, n):
    return jax.ops.segment_sum(src, seg, n)

class _Rng:

    def __init__(self, key):
        self._k = key

    def _next(self):
        self._k, sub = jax.random.split(self._k)
        return sub

    def normal(self, shape):
        return jax.random.normal(self._next(), shape, dtype=jnp.bfloat16)

    def randint(self, lo, hi, shape):
        return jax.random.randint(self._next(), shape, lo, hi, dtype=jnp.int32)

    def uniform(self, shape, lo=0.0, hi=1.0):
        return jax.random.uniform(self._next(), shape, jnp.bfloat16, lo, hi)

    def permutation(self, n):
        return jax.random.permutation(self._next(), n)
kernel_name = 'parallel_sum__memory_aug_recurrent_mem_tr__dense_activation_silu__prompt'

def setup_inputs():
    _rng = _Rng(jax.random.key(int.from_bytes(__import__("os").urandom(4), "little")))
    _w = lambda a: (lambda t: t.astype(jnp.bfloat16) if jnp.issubdtype(t.dtype, jnp.floating) else t)(jnp.asarray(a))

    def _A_setup():
        B, S, Dm = (1, 2048, 448)
        H, Dh = (16, 256)
        M, seg = (8, 32)
        seg = min(seg, S)
        S = S // seg * seg
        return {'x': _w((lambda *s: _rng.normal(s) * 0.05)(B, S, Dm)), 'mem0': _w((lambda *s: _rng.normal(s) * 0.2)(B, M, Dm)), 'Wq': _w((lambda *s: _rng.normal(s) * 0.8)(Dm, H, Dh) * Dm ** (-0.5)), 'Wk': _w((lambda *s: _rng.normal(s) * 0.8)(Dm, H, Dh) * Dm ** (-0.5)), 'Wv': _w((lambda *s: _rng.normal(s) * 0.2)(Dm, H, Dh) * Dm ** (-0.5)), 'Wo': _w((lambda *s: _rng.normal(s) * 0.2)(H, Dh, Dm) * (H * Dh) ** (-0.5)), 'seg_len': seg}
    _A_in = _A_setup()

    def _B_setup():
        B, S, D, F = (1, 2048, 448, 1792)
        return {'x': _w((lambda *s: _rng.normal(s) * 0.05)(B, S, D)), 'w1': _w((lambda *s: _rng.normal(s) * 0.05)(D, F) * D ** (-0.5)), 'w2': _w((lambda *s: _rng.normal(s) * 0.05)(F, D) * F ** (-0.5))}
    _B_in = _B_setup()
    return {'A_x': _A_in['x'], 'A_mem0': _A_in['mem0'], 'A_Wq': _A_in['Wq'], 'A_Wk': _A_in['Wk'], 'A_Wv': _A_in['Wv'], 'A_Wo': _A_in['Wo'], 'A_seg_len': _A_in['seg_len'], 'B_x': _B_in['x'], 'B_w1': _B_in['w1'], 'B_w2': _B_in['w2']}

def reference(A_x, A_mem0, A_Wq, A_Wk, A_Wv, A_Wo, A_seg_len, B_x, B_w1, B_w2):

    def _A_ref(x, mem0, Wq, Wk, Wv, Wo, seg_len):
        B, S, Dm = x.shape
        H, Dh = (Wq.shape[1], Wq.shape[2])
        M = mem0.shape[1]
        scale = Dh ** (-0.5)
        n_seg = S // seg_len
        L = M + seg_len
        idx = jnp.arange(L)
        mask = (idx[:, None] < M) | (idx[:, None] >= idx[None, :])
        mem = mem0
        outs = []
        for s in range(n_seg):
            xs = x[:, s * seg_len:(s + 1) * seg_len, :].copy()
            h = jnp.concatenate([mem, xs], axis=1)
            q = jnp.einsum('btd,dhe->bhte', h, Wq)
            k = jnp.einsum('btd,dhe->bhte', h, Wk)
            v = jnp.einsum('btd,dhe->bhte', h, Wv)
            scores = jnp.einsum('bhqe,bhke->bhqk', q, k) * scale
            scores = jnp.where(mask[None, None], scores, -1000000000.0)
            p = _softmax(scores, axis=-1)
            o = jnp.einsum('bhqk,bhke->bhqe', p, v)
            o = jnp.einsum('bhte,hed->btd', o, Wo)
            mem = o[:, :M, :].copy()
            outs.append(o[:, M:, :])
        return jnp.concatenate(outs, axis=1)

    def _B_ref(x, w1, w2):
        h = jnp.einsum('bsd,df->bsf', x, w1)
        h = _silu(h)
        out = jnp.einsum('bsf,fd->bsd', h, w2)
        return out
    x = A_x
    xn = _layernorm(x, axis=-1)
    return x + _A_ref(xn, A_mem0, A_Wq, A_Wk, A_Wv, A_Wo, A_seg_len) + _B_ref(xn, B_w1, B_w2)
```

```python
import functools
import jax
import jax.numpy as jnp
from jax import lax
import jax.experimental.pallas as pl
import jax.experimental.pallas.tpu as pltpu

S, D, H, E, F, M, SEG = 2048, 448, 16, 256, 1792, 8, 32
NSEG = S // SEG
L = M + SEG
EPS = 1e-5
SCALE = E ** -0.5
TB = 128
NB = S // TB
f32, bf16, u32 = jnp.float32, jnp.bfloat16, jnp.uint32

def _bf(u):
    return pltpu.bitcast(u, bf16)

def _dot(a, b):
    return lax.dot_general(a, b, (((1,), (0,)), ((), ())), preferred_element_type=f32)

def _dot_nt(a, b):
    return lax.dot_general(a, b, (((1,), (1,)), ((), ())), preferred_element_type=f32)


def _kernel(xT_hbm, mem_hbm, wq_hbm, wk_hbm, wv_hbm, woT_hbm, w1_hbm, w2T_hbm, oT_hbm,
            xT, membuf, wraw, wqkv, woT, w1, w2T, xn, hid, oacc, astage, obuf,
            sems, wsems, osems):
    cx = pltpu.make_async_copy(xT_hbm, xT, sems.at[0]); cx.start()
    c1 = pltpu.make_async_copy(w1_hbm.bitcast(u32), w1, sems.at[1]); c1.start()
    cm = pltpu.make_async_copy(mem_hbm, membuf, sems.at[2]); cm.start()
    srcs = [wq_hbm.bitcast(u32), wk_hbm.bitcast(u32), wv_hbm.bitcast(u32)]
    wcp = {}
    for hp in range(H // 2):
        for j in range(3):
            c = pltpu.make_async_copy(srcs[j].at[:, hp, :], wraw.at[j, hp], wsems.at[j, hp]); c.start()
            wcp[(j, hp)] = c
    co = pltpu.make_async_copy(woT_hbm.bitcast(u32), woT, sems.at[3]); co.start()
    c2 = pltpu.make_async_copy(w2T_hbm.bitcast(u32), w2T, sems.at[4]); c2.start()

    cx.wait(); c1.wait()

    def ln_body(b, c):
        r = pl.multiple_of(b * TB, TB)
        xv = xT[:, pl.ds(r, TB)].astype(f32)
        m = jnp.mean(xv, axis=0, keepdims=True)
        xc = xv - m
        var = jnp.mean(xc * xc, axis=0, keepdims=True)
        xnT = xc * lax.rsqrt(var + EPS)
        xnv = xnT.T
        xn[pl.ds(r, TB), :] = xnv
        h1 = _dot(xnv.astype(bf16), _bf(w1[...]))
        hid[pl.ds(r, TB), :] = (h1 * jax.nn.sigmoid(h1)).astype(bf16)
        return c
    lax.fori_loop(0, NB, ln_body, 0)

    for hp in range(H // 2):
        for j in range(3):
            wcp[(j, hp)].wait()
            u = wraw[j, hp]
            for t in range(2):
                val = pltpu.unpack_elementwise(u, index=t, packed_dtype=bf16, unpacked_dtype=f32)
                col = (2 * hp + t) * 3 * E + j * E
                wqkv[:, col:col + E] = pltpu.bitcast(val.astype(bf16), u32)
    co.wait(); c2.wait(); cm.wait()

    row = lax.broadcasted_iota(jnp.int32, (L, L), 0)
    col = lax.broadcasted_iota(jnp.int32, (L, L), 1)
    mask = (row < M) | (row >= col)

    def step(s, mem):
        r = pl.multiple_of(s * SEG, SEG)
        hcat = jnp.concatenate([mem, xn[pl.ds(r, SEG), :]], axis=0)
        st = {}
        def qkv_stage(hd):
            qkv = _dot(hcat, _bf(wqkv[:, hd * 3 * E:(hd + 1) * 3 * E]))
            st[hd] = (qkv[:, :E], qkv[:, E:2 * E].astype(bf16), qkv[:, 2 * E:].astype(bf16))
        def s_stage(hd):
            q, k, v = st[hd]
            sc = _dot_nt(q, k) * SCALE
            sc = jnp.where(mask, sc, -1e9)
            mx = jnp.max(sc, axis=-1, keepdims=True)
            p = jnp.exp(sc - mx)
            p = p * pl.reciprocal(jnp.sum(p, axis=-1, keepdims=True), approx=True)
            st[hd] = (p, v)
        def pv_stage(hd):
            p, v = st[hd]
            st[hd] = _dot(p, v)
        acc = [None]
        def o_stage(hd):
            t = _dot_nt(st[hd], _bf(woT[hd * (D // 2):(hd + 1) * (D // 2), :]))
            acc[0] = t if acc[0] is None else acc[0] + t
        LS, LP, LO = 1, 2, 3
        for i in range(H + LO):
            if i < H: qkv_stage(i)
            if 0 <= i - LP < H: pv_stage(i - LP)
            if 0 <= i - LO < H: o_stage(i - LO)
            if 0 <= i - LS < H: s_stage(i - LS)
        a = acc[0]
        b = s // 4
        j = s % 4
        rq = pl.multiple_of(j * (D // 8), D // 8)
        hb = hid[pl.ds(pl.multiple_of(b * TB, TB), TB), :]
        f2 = _dot_nt(_bf(w2T[pl.ds(rq, D // 8), :]), hb)
        ro = pl.multiple_of(j * (D // 4), D // 4)
        oacc[b, pl.ds(ro, D // 4), :] = f2
        astage[b, pl.ds(pl.multiple_of(j * SEG, SEG), SEG), :] = a[M:, :]
        return a[:M, :]

    lax.fori_loop(0, NSEG, step, membuf[...].astype(f32))

    def out_body(b, c):
        r = pl.multiple_of(b * TB, TB)
        at = astage[b].T
        res = xT[:, pl.ds(r, TB)].astype(f32) + oacc[b] + at
        slot = b % 2
        @pl.when(b >= 2)
        def _():
            pltpu.make_async_copy(obuf.at[slot], oT_hbm.at[:, pl.ds(0, TB)], osems.at[slot]).wait()
        obuf[slot] = res.astype(bf16)
        pltpu.make_async_copy(obuf.at[slot], oT_hbm.at[:, pl.ds(r, TB)], osems.at[slot]).start()
        return c
    lax.fori_loop(0, NB, out_body, 0)
    for slot in range(2):
        pltpu.make_async_copy(obuf.at[slot], oT_hbm.at[:, pl.ds(0, TB)], osems.at[slot]).wait()


@jax.jit
def pallas_parallel_sum__memory_aug_recurrent_mem_tr__dense_activation_silu__prompt_kernel(A_x, A_mem0, A_Wq, A_Wk, A_Wv, A_Wo, A_seg_len, B_x, B_w1, B_w2):
    xT = A_x.reshape(S, D).T
    mem0 = A_mem0.reshape(M, D)
    woT = A_Wo.transpose(0, 2, 1).reshape(H * D, E)
    w2T = B_w2.T
    hbm = pl.BlockSpec(memory_space=pltpu.HBM)
    outT = pl.pallas_call(
        _kernel,
        out_shape=jax.ShapeDtypeStruct((D, S), A_x.dtype),
        in_specs=[hbm] * 8,
        out_specs=hbm,
        scratch_shapes=[
            pltpu.VMEM((D, S), bf16),
            pltpu.VMEM((M, D), bf16),
            pltpu.VMEM((3, H // 2, D, E), u32),
            pltpu.VMEM((D // 2, 3 * H * E), u32),
            pltpu.VMEM((H * D // 2, E), u32),
            pltpu.VMEM((D // 2, F), u32),
            pltpu.VMEM((D // 2, F), u32),
            pltpu.VMEM((S, D), f32),
            pltpu.VMEM((S, F), bf16),
            pltpu.VMEM((NB, D, TB), f32),
            pltpu.VMEM((NB, TB, D), f32),
            pltpu.VMEM((2, D, TB), bf16),
            pltpu.SemaphoreType.DMA((5,)),
            pltpu.SemaphoreType.DMA((3, H // 2)),
            pltpu.SemaphoreType.DMA((2,)),
        ],
        compiler_params=pltpu.CompilerParams(vmem_limit_bytes=100 * 1024 * 1024),
    )(xT, mem0, A_Wq, A_Wk, A_Wv, woT, B_w1, w2T)
    return outT.T.reshape(1, S, D)
```

```python
import functools
import jax
import jax.numpy as jnp
from jax import lax
import jax.experimental.pallas as pl
import jax.experimental.pallas.tpu as pltpu

S, D, H, E, F, M, SEG = 2048, 448, 16, 256, 1792, 8, 32
NSEG = S // SEG
L = M + SEG
EPS = 1e-5
SCALE = E ** -0.5
LOG2E = 1.4426950408889634
TB = 128
NB = S // TB
NSTEPS = NSEG
HP = H // 2
f32, bf16, u32 = jnp.float32, jnp.bfloat16, jnp.uint32
NN = (((1,), (0,)), ((), ()))
NT = (((1,), (1,)), ((), ()))

def _bf(u):
    return pltpu.bitcast(u, bf16)

def _u(b):
    return pltpu.bitcast(b, u32)


def _kernel(xT_hbm, mem_hbm, wq_hbm, wk_hbm, wv_hbm, woT_hbm, w1_hbm, w2T_hbm, oT_hbm,
            xT, membuf, wraw, wqkv, woT, wo, w1, w2T, xn, w2f, hlast, hidT, oacc, astage, obuf,
            sems, xsems, wsems, osems):
    XC = 4
    XW = S // XC
    cm = pltpu.make_async_copy(mem_hbm, membuf, sems.at[2]); cm.start()
    def xcopy(i):
        return pltpu.make_async_copy(xT_hbm.at[:, pl.ds(i * XW, XW)], xT.at[:, pl.ds(i * XW, XW)], xsems.at[i])
    for i in range(XC):
        xcopy(i).start()
    c1 = pltpu.make_async_copy(w1_hbm.bitcast(u32), w1, sems.at[1]); c1.start()
    srcs = [wq_hbm.bitcast(u32), wk_hbm.bitcast(u32), wv_hbm.bitcast(u32)]
    def wcopy(j, hp):
        return pltpu.make_async_copy(srcs[j].at[:, hp, :], wraw.at[j, hp], wsems.at[j, hp])
    woT_u = woT_hbm.bitcast(u32)
    HR = H * D // 4
    def ocopy(i):
        return pltpu.make_async_copy(woT_u.at[pl.ds(i * HR, HR), :], woT.at[pl.ds(i * HR, HR), :], sems.at[3 + i])
    ocopy(0).start(); ocopy(1).start()
    for hp in range(HP):
        for j in range(3):
            wcopy(j, hp).start()
    c2 = pltpu.make_async_copy(w2T_hbm.bitcast(u32), w2T, sems.at[0]); c2.start()
    astage[...] = jnp.zeros_like(astage)
    oacc[1] = jnp.zeros_like(oacc[1])

    LNU = XW // TB
    def ln_body(i, c):
        pltpu.make_async_copy(xT_hbm.at[:, pl.ds(0, XW)], xT.at[:, pl.ds(0, XW)], xsems.at[i]).wait()
        for t in range(LNU):
            b = i * LNU + t
            r = pl.multiple_of(b * TB, TB)
            xv = xT[:, pl.ds(r, TB)].astype(f32)
            m = jnp.mean(xv, axis=0, keepdims=True)
            xc = xv - m
            var = jnp.mean(xc * xc, axis=0, keepdims=True)
            xnv = (xc * lax.rsqrt(var + EPS)).T
            xn[pl.ds(r, TB), :] = xnv
        return c
    lax.fori_loop(0, NB // LNU, ln_body, 0)

    def relayout_piece(hp, j, r0, nr):
        u = wraw[j, hp, pl.ds(r0, nr), :]
        for t in range(2):
            val = pltpu.unpack_elementwise(u, index=t, packed_dtype=bf16, unpacked_dtype=f32)
            ro = pl.multiple_of((2 * hp + t) * (D // 2) + r0 // 2, 8)
            wqkv[pl.ds(ro, nr // 2), j * E:(j + 1) * E] = _u(val.astype(bf16))

    def relayout(hp):
        for j in range(3):
            wcopy(j, hp).wait()
        for j in range(3):
            for r0 in range(0, D, 64):
                relayout_piece(hp, j, r0, 64)

    def finish(b, c, h1):
        hv = h1 * pl.reciprocal(1.0 + jnp.exp2(h1 * (-LOG2E)), approx=True)
        hidT[b, c * 64:(c + 1) * 64, :] = _u(hv.T.astype(bf16))

    def wo_head(hd):
        wt = _bf(woT[pl.ds(pl.multiple_of(hd * (D // 2), D // 2), D // 2), :]).astype(f32)
        wo[pl.ds(pl.multiple_of(hd * (E // 2), E // 2), E // 2), :] = _u(wt.T.astype(bf16))

    NC = F // 128
    def ffn1(i, hp=None, first=None):
        pieces = []
        if hp is not None:
            for j in range(3):
                wcopy(j, hp).wait()
            pieces = [(j, r0) for j in range(3) for r0 in range(0, D, 32)]
        nd = 2 * NC - 8
        prev = None
        if first is None:
            prev = (2 * i - 1, NC - 1, hlast[...])
        for t in range(2):
            b = 2 * i + t
            lhs = xn[pl.ds(pl.multiple_of(b * TB, TB), TB), :]
            for c in range(NC):
                h1 = lax.dot_general(lhs, _bf(w1[:, c * 128:(c + 1) * 128]), NN, preferred_element_type=f32)
                if prev is not None:
                    finish(*prev)
                n = t * NC + c
                if hp is not None and n in (6, 13, 20):
                    wo_head(3 * hp + (n - 6) // 7)
                for (j, r0) in pieces[min(n, nd) * len(pieces) // nd:min(n + 1, nd) * len(pieces) // nd]:
                    relayout_piece(hp, j, r0, 32)
                prev = (b, c, h1)
        hlast[...] = prev[2]

    c1.wait()
    NA = 3
    ffn1(0, None, True)
    def f1a_body(i, c):
        ffn1(i)
        return c
    lax.fori_loop(1, NA, f1a_body, 0)
    ocopy(0).wait(); ocopy(1).wait()
    def f1b_body(i, c):
        ffn1(i, i - NA)
        return c
    lax.fori_loop(NA, NB // 2, f1b_body, 0)
    finish(NB - 1, NC - 1, hlast[...])

    def rl_body(hp, c):
        relayout(hp)
        return c
    lax.fori_loop(NB // 2 - NA, HP, rl_body, 0)
    wo_head(H - 1)
    c2.wait(); cm.wait()
    def w2_body(i, c):
        r = pl.multiple_of(i * 32, 32)
        w2f[pl.ds(r, 32), :] = _bf(w2T[pl.ds(pl.multiple_of(i * 16, 16), 16), :]).astype(f32)
        return c
    lax.fori_loop(0, D // 32, w2_body, 0)

    row = lax.broadcasted_iota(jnp.int32, (L, L), 0)
    col = lax.broadcasted_iota(jnp.int32, (L, L), 1)
    mask = (row < M) | (row >= col)

    def finish_block(b, slot):
        r = pl.multiple_of(b * TB, TB)
        at = astage[slot].T
        res = xT[:, pl.ds(r, TB)].astype(f32) + oacc[slot] + at
        obuf[slot] = res.astype(bf16)

    def out_copy(b, slot):
        return pltpu.make_async_copy(obuf.at[slot], oT_hbm.at[:, pl.ds(pl.multiple_of(b * TB, TB), TB)], osems.at[slot])

    def step(b, slot, j, mem):
        r = pl.multiple_of(b * TB + j * SEG, SEG)
        hcat = jnp.concatenate([mem, xn[pl.ds(r, SEG), :]], axis=0)
        st = {}
        def qkv_stage(hd):
            qkv = lax.dot_general(hcat, _bf(wqkv[hd * (D // 2):(hd + 1) * (D // 2), :]), NN, preferred_element_type=f32)
            st[hd] = (qkv[:, :E], qkv[:, E:2 * E].astype(bf16), qkv[:, 2 * E:].astype(bf16))
        def s_stage(hd):
            q, k, v = st[hd]
            sc = lax.dot_general(q, k, NT, preferred_element_type=f32) * SCALE
            sc = jnp.where(mask, sc, -1e9)
            mx = jnp.max(sc, axis=-1, keepdims=True)
            p = jnp.exp(sc - mx)
            p = p * pl.reciprocal(jnp.sum(p, axis=-1, keepdims=True), approx=True)
            st[hd] = (p, v)
        def pv_stage(hd):
            p, v = st[hd]
            st[hd] = lax.dot_general(p, v, NN, preferred_element_type=f32)
        acc = [None]
        def o_stage(g):
            o2 = jnp.concatenate([st[2 * g], st[2 * g + 1]], axis=1)
            t = lax.dot_general(o2, _bf(wo[g * E:(g + 1) * E, :]), NN, preferred_element_type=f32)
            acc[0] = t if acc[0] is None else acc[0] + t
        def ffn2(lo, hi):
            n = hi - lo
            f2 = lax.dot_general(w2f[pl.ds(j * (D // 4) + lo, n), :], _bf(hidT[b]), NN, preferred_element_type=f32)
            oacc[slot, pl.ds(j * (D // 4) + lo, n), :] = f2
        for g in range(HP):
            qkv_stage(2 * g); qkv_stage(2 * g + 1)
            if g >= 1:
                s_stage(2 * g - 2); s_stage(2 * g - 1)
            if g >= 2:
                pv_stage(2 * g - 4); pv_stage(2 * g - 3)
            if g >= 3:
                o_stage(g - 3)
        s_stage(H - 2); s_stage(H - 1)
        o_stage(HP - 3)
        pv_stage(H - 4); pv_stage(H - 3)
        ffn2(0, 32)
        o_stage(HP - 2)
        pv_stage(H - 2); pv_stage(H - 1)
        ffn2(32, 64)
        o_stage(HP - 1)
        ffn2(64, 112)
        a = acc[0]
        astage[slot, pl.ds(j * SEG, SEG), :] = a[M:, :]
        return a[:M, :]

    def block(b, mem):
        slot = b % 2
        @pl.when(b >= 3)
        def _():
            out_copy(b - 3, 1 - slot).wait()
        finish_block(jnp.maximum(b - 1, 0), 1 - slot)
        for j in range(4):
            mem = step(b, slot, j, mem)
        @pl.when(b >= 1)
        def _():
            out_copy(b - 1, 1 - slot).start()
        return mem
    lax.fori_loop(0, NSTEPS // 4, block, membuf[...].astype(f32))

    nb = NSTEPS // 4
    sl = (nb - 1) % 2
    out_copy(nb - 3, sl).wait()
    finish_block(nb - 1, sl)
    out_copy(nb - 1, sl).start()
    out_copy(nb - 2, 1 - sl).wait()
    out_copy(nb - 1, sl).wait()


@jax.jit
def pallas_parallel_sum__memory_aug_recurrent_mem_tr__dense_activation_silu__prompt_kernel(A_x, A_mem0, A_Wq, A_Wk, A_Wv, A_Wo, A_seg_len, B_x, B_w1, B_w2):
    xT = A_x.reshape(S, D).T
    mem0 = A_mem0.reshape(M, D)
    woT = A_Wo.transpose(0, 2, 1).reshape(H * D, E)
    w2T = B_w2.T
    hbm = pl.BlockSpec(memory_space=pltpu.HBM)
    outT = pl.pallas_call(
        _kernel,
        out_shape=jax.ShapeDtypeStruct((D, S), A_x.dtype),
        in_specs=[hbm] * 8,
        out_specs=hbm,
        scratch_shapes=[
            pltpu.VMEM((D, S), bf16),
            pltpu.VMEM((M, D), bf16),
            pltpu.VMEM((3, HP, D, E), u32),
            pltpu.VMEM((H * D // 2, 3 * E), u32),
            pltpu.VMEM((H * D // 2, E), u32),
            pltpu.VMEM((H * E // 2, D), u32),
            pltpu.VMEM((D // 2, F), u32),
            pltpu.VMEM((D // 2, F), u32),
            pltpu.VMEM((S, D), f32),
            pltpu.VMEM((D, F), f32),
            pltpu.VMEM((TB, 128), f32),
            pltpu.VMEM((NB, F // 2, TB), u32),
            pltpu.VMEM((2, D, TB), f32),
            pltpu.VMEM((2, TB, D), f32),
            pltpu.VMEM((2, D, TB), bf16),
            pltpu.SemaphoreType.DMA((5,)),
            pltpu.SemaphoreType.DMA((4,)),
            pltpu.SemaphoreType.DMA((3, HP)),
            pltpu.SemaphoreType.DMA((2,)),
        ],
        compiler_params=pltpu.CompilerParams(vmem_limit_bytes=100 * 1024 * 1024),
    )(xT, mem0, A_Wq, A_Wk, A_Wv, woT, B_w1, w2T)
    return outT.T.reshape(1, S, D)
```

```python
import functools

import jax
import jax.numpy as jnp
from jax import lax
import jax.experimental.pallas as pl
import jax.experimental.pallas.tpu as pltpu

S, D, H, E, F, M, SEG = 2048, 448, 16, 256, 1792, 8, 32
L = M + SEG
HP = H // 2
TB = 128
NB = S // TB
DH = D // 2
DM = 192
NC = F // 128
NA, NM = 4, 10
EPS = 1e-5
SCALE = E ** -0.5
LOG2E = 1.4426950408889634
NSTEPS = S // SEG

T_NT = {t: sorted({(g // 5) // 2 for g in range(16 * t, 16 * t + 16)}) for t in range(5)}
T_LAST = {n: max(t for t in T_NT if n in T_NT[t]) for n in range(HP)}

ORDER = (
    "Q0 Q1 Q2 Q3 S0 S1 Q4 Q5 S2 S3 X0 Q6 Q7 S4 S5 X1 Q8 Q9 S6 S7 T0 X2 Q10 Q11 S8 S9 X3 "
    "Q12 Q13 S10 S11 T1 X4 Q14 Q15 S12 S13 T2 S14 X5 S15 X6 X7 U0:4 P0:2 P2:4 T3 T4 "
    "F0:64 U4:6 U6:8 P4:5 F64:112"
).split()

f32, bf16, u32 = jnp.float32, jnp.bfloat16, jnp.uint32
NN = (((1,), (0,)), ((), ()))
NT = (((1,), (1,)), ((), ()))


def _bf(words):
    return pltpu.bitcast(words, bf16)


def _u(vals):
    return pltpu.bitcast(vals, u32)


def _mm(a, b, dims=NN):
    return lax.dot_general(a, b, dims, preferred_element_type=f32)


def _unpack(words, half):
    return pltpu.unpack_elementwise(words, index=half, packed_dtype=bf16, unpacked_dtype=f32)


def _kernel(xT_hbm, mem_hbm, wq_hbm, wk_hbm, wv_hbm, woT_hbm, w1_hbm, w2T_hbm, oT_hbm,
            xT, membuf, wraw, wqk, woT, wb, w1, w2T, xn, hlast, pall, vw, hbuf, tbuf, wtl, hidT, oacc, astage, obuf, sems, xsems, wsems, osems):
    w1_u, woT_u = w1_hbm.bitcast(u32), woT_hbm.bitcast(u32)
    wsrc = [w.bitcast(u32) for w in (wq_hbm, wk_hbm, wv_hbm)]

    def x_copy(i):
        cols = (pl.ds(0, NA * TB), pl.ds(NA * TB, (NM - NA) * TB), pl.ds(NM * TB, S - NM * TB))[i]
        return pltpu.make_async_copy(xT_hbm.at[:, cols], xT.at[:, cols], xsems.at[i])

    def w1_copy(i):
        cols = pl.ds(i * (F // 2), F // 2)
        return pltpu.make_async_copy(w1_u.at[:, cols], w1.at[:, cols], sems.at[1 + 2 * i])

    def w_copy(j, g):
        return pltpu.make_async_copy(wsrc[j].at[:, g, :], wraw.at[j, g], wsems.at[j, g])

    def wo_copy(g):
        rows = pl.ds(pl.multiple_of(g * D, 8), D)
        return pltpu.make_async_copy(woT_u.at[rows, :], woT.at[rows, :], wsems.at[3, g])

    def pair_wait(g):
        wo_copy(g).wait()
        for j in range(3):
            w_copy(j, g).wait()

    mem_copy = pltpu.make_async_copy(mem_hbm, membuf, sems.at[2])
    w2_copy = pltpu.make_async_copy(w2T_hbm.bitcast(u32), w2T, sems.at[0])
    mem_copy.start()
    x_copy(0).start()
    w1_copy(0).start()
    w1_copy(1).start()
    x_copy(1).start()
    x_copy(2).start()
    for g in range(HP):
        wo_copy(g).start()
        for j in (2, 0, 1):
            w_copy(j, g).start()
    w2_copy.start()
    astage[...] = jnp.zeros_like(astage)
    oacc[1] = jnp.zeros_like(oacc[1])

    def ln_block(b):
        xv = xT[:, b * TB:(b + 1) * TB].astype(f32)
        xc = xv - jnp.mean(xv, axis=0, keepdims=True)
        var = jnp.mean(xc * xc, axis=0, keepdims=True)
        xn[b * TB:(b + 1) * TB, :] = (xc * lax.rsqrt(var + EPS)).T

    def ffn1_finish(b, c, h1):
        hv = h1 * pl.reciprocal(1.0 + jnp.exp2(h1 * (-LOG2E)), approx=True)
        hidT[b, c * 64:(c + 1) * 64, :] = _u(hv.T.astype(bf16))

    def ffn1(tiles, items=(), prev=None):
        for n, (b, c) in enumerate(tiles):
            if c == tiles[0][1] or n == 0:
                lhs = xn[pl.ds(pl.multiple_of(b * TB, TB), TB), :]
            h1 = _mm(lhs, _bf(w1[:, c * 128:(c + 1) * 128]))
            if prev is not None:
                ffn1_finish(*prev)
            for item in items[n * len(items) // len(tiles):(n + 1) * len(items) // len(tiles)]:
                item()
            prev = (b, c, h1)
        hlast[...] = prev[2]
        return prev[:2]

    def pair_items(g):
        items = []
        for t in range(2):
            ro = pl.multiple_of((2 * g + t) * DH, 8)
            for m in range(2):

                def retile_qk(t=t, m=m, ro=ro):
                    for j in range(2):
                        val = _unpack(wraw[j, g, m * DH:(m + 1) * DH, :], t)
                        wqk[pl.ds(ro + m * (DH // 2), DH // 2), j * E:(j + 1) * E] = _u(val.astype(bf16))

                def fold(n, t=t, m=m, ro=ro):
                    wv = _unpack(wraw[2, g, m * DH:(m + 1) * DH, :], t)
                    wo = _bf(woT[pl.ds(ro + n * 64, 64 if n < 3 else 32), :])
                    bu = _u(_mm(wv, wo, NT).astype(bf16))
                    if n < 3:
                        cb, ct = slice(t * 384 + n * 128, t * 384 + (n + 1) * 128), slice(n * 128, (n + 1) * 128)
                    else:
                        cb, ct = slice(768 + t * 64, 768 + (t + 1) * 64), slice(384, D)
                    rb = pl.multiple_of(g * DM, 8)
                    if m == 0:
                        wb[pl.ds(rb, DH // 2), cb] = bu
                    else:
                        nm = DM - DH // 2
                        wb[pl.ds(rb + DH // 2, nm), cb] = bu[:nm]
                        wtl[pl.ds(pl.multiple_of(g * 64, 8) + 32 * t, 32), ct] = bu[nm:]

                items.append(retile_qk)
                items.extend(functools.partial(fold, n) for n in range(4))
        return items

    lo, hi, both = range(NC // 2), range(NC // 2, NC), range(NC)
    x_copy(0).wait()
    for b in range(NA):
        ln_block(b)
    w1_copy(0).wait()
    last = ffn1([(b, c) for b in (0, 1) for c in lo])
    w1_copy(1).wait()
    ffn1_finish(*last, hlast[...])
    last = ffn1([(b, c) for b in (0, 1) for c in hi])
    x_copy(1).wait()
    ffn1_finish(*last, hlast[...])
    last = ffn1([(2, c) for c in both], [functools.partial(ln_block, b) for b in range(NA, NM)])
    x_copy(2).wait()
    ffn1_finish(*last, hlast[...])
    ffn1([(3, c) for c in both], [functools.partial(ln_block, b) for b in range(NM, NB)])

    def prologue_body(i, carry):
        pair_wait(i - 2)
        ffn1([(2 * i + t, c) for t in range(2) for c in both], pair_items(i - 2),
             prev=(2 * i - 1, NC - 1, hlast[...]))
        return carry

    lax.fori_loop(2, NB // 2, prologue_body, 0)
    pair_wait(HP - 2)
    pair_wait(HP - 1)
    ffn1_finish(NB - 1, NC - 1, hlast[...])
    for item in pair_items(HP - 2) + pair_items(HP - 1):
        item()
    w2_copy.wait()
    mem_copy.wait()

    row = lax.broadcasted_iota(jnp.int32, (L, L), 0)
    col = lax.broadcasted_iota(jnp.int32, (L, L), 1)
    mask = (row < M) | (row >= col)

    def step(b, slot, j, mem):
        hbuf[0:M, :] = mem
        hbuf[M:L, :] = xn[pl.ds(pl.multiple_of(b * TB + j * SEG, SEG), SEG), :]
        ht = hbuf[:, 2 * DM:D]
        ht_lane = (jnp.concatenate([ht, jnp.zeros_like(ht)], axis=1),
                   jnp.concatenate([jnp.zeros_like(ht), ht], axis=1))
        zero8 = jnp.zeros((8, 128), f32)
        qk, tacc, acc = {}, {}, []

        def qk_proj(h):
            r = _mm(hbuf[...], _bf(wqk[h * DH:(h + 1) * DH, :]))
            qk[h] = (r[:, :E], r[:, E:].astype(bf16))

        def softmax(h):
            q, k = qk[h]
            sc = jnp.where(mask, _mm(q, k, NT) * SCALE, -1e9)
            p = jnp.exp(sc - jnp.max(sc, axis=-1, keepdims=True))
            pall[:, h * L:(h + 1) * L] = p * pl.reciprocal(jnp.sum(p, axis=-1, keepdims=True), approx=True)

        def value_main(g):
            hb = _mm(hbuf[:, 0:2 * DM], _bf(wb[g * DM:(g + 1) * DM, :]))
            va = jnp.concatenate([hb[:, 0:384], hb[:, 768:832]], axis=1)
            vb = jnp.concatenate([hb[:, 384:768], hb[:, 832:896]], axis=1)
            vw[g * L:(g + 1) * L, :] = _u(jnp.concatenate([va, vb], axis=0).astype(bf16))

        def t_tile(t):
            cols = []
            for n in T_NT[t]:
                rows = []
                for g in range(16 * t, 16 * t + 16):
                    h, k = g // 5, g % 5
                    rows.append(ht_lane[h % 2][8 * k:8 * k + 8] if h // 2 == n else zero8)
                cols.append(jnp.concatenate(rows, axis=0))
            r = _mm(pall[:, t * 128:(t + 1) * 128], jnp.concatenate(cols, axis=1).astype(bf16))
            for i, n in enumerate(T_NT[t]):
                part = r[:, i * 128:(i + 1) * 128]
                tacc[n] = tacc[n] + part if n in tacc else part
                if T_LAST[n] == t:
                    tbuf[:, n * 128:(n + 1) * 128] = tacc[n]

        def accumulate(r):
            acc[:] = [acc[0] + r if acc else r]

        def p_tiles(t0, t1):
            accumulate(_mm(pall[:, t0 * 128:t1 * 128], _bf(vw[t0 * 64:t1 * 64, :])))

        def u_tiles(g0, g1):
            accumulate(_mm(tbuf[:, g0 * 128:g1 * 128], _bf(wtl[g0 * 64:g1 * 64, :])))

        def ffn2(r0, r1):
            w = _bf(w2T[pl.ds((j * (D // 4) + r0) // 2, (r1 - r0) // 2), :])
            oacc[slot, pl.ds(j * (D // 4) + r0, r1 - r0), :] = _mm(w, _bf(hidT[b]))

        ops = dict(Q=qk_proj, S=softmax, X=value_main, T=t_tile, P=p_tiles, U=u_tiles, F=ffn2)
        for op in ORDER:
            ops[op[0]](*(int(v) for v in op[1:].split(":")))
        out = acc[0]
        astage[slot, pl.ds(j * SEG, SEG), :] = out[M:, :]
        return out[:M, :]

    def finish_block(b, slot, oslot):
        xb = xT[:, pl.ds(pl.multiple_of(b * TB, TB), TB)].astype(f32)
        obuf[oslot] = (xb + oacc[slot] + astage[slot].T).astype(bf16)

    def out_copy(b):
        cols = pl.ds(pl.multiple_of(b * TB, TB), TB)
        return pltpu.make_async_copy(obuf.at[b % 4], oT_hbm.at[:, cols], osems.at[b % 4])

    def two_blocks(i, mem):
        b = 2 * i

        @pl.when(i >= 2)
        def _():
            out_copy(b - 4).wait()

        @pl.when(i >= 3)
        def _():
            out_copy(b - 5).wait()

        finish_block(jnp.maximum(b - 1, 0), 1, (b + 3) % 4)
        for j in range(4):
            mem = step(b, 0, j, mem)
        finish_block(b, 0, b % 4)
        for j in range(4):
            mem = step(b + 1, 1, j, mem)

        @pl.when(i >= 1)
        def _():
            out_copy(b - 1).start()

        out_copy(b).start()
        return mem

    lax.fori_loop(0, NSTEPS // 8, two_blocks, membuf[...].astype(f32))

    nb = NSTEPS // 4
    out_copy(nb - 5).wait()
    finish_block(nb - 1, 1, (nb - 1) % 4)
    out_copy(nb - 1).start()
    for b in range(nb - 4, nb):
        out_copy(b).wait()


@jax.jit
def pallas_parallel_sum__memory_aug_recurrent_mem_tr__dense_activation_silu__prompt_kernel(A_x, A_mem0, A_Wq, A_Wk, A_Wv, A_Wo, A_seg_len, B_x, B_w1, B_w2):
    del A_seg_len, B_x
    hbm = pl.BlockSpec(memory_space=pltpu.HBM)
    outT = pl.pallas_call(
        _kernel,
        out_shape=jax.ShapeDtypeStruct((D, S), A_x.dtype),
        in_specs=[hbm] * 8,
        out_specs=hbm,
        scratch_shapes=[
            pltpu.VMEM((D, S), bf16),
            pltpu.VMEM((M, D), bf16),
            pltpu.VMEM((3, HP, D, E), u32),
            pltpu.VMEM((H * DH, 2 * E), u32),
            pltpu.VMEM((H * DH, E), u32),
            pltpu.VMEM((HP * DM, 2 * D), u32),
            pltpu.VMEM((DH, F), u32),
            pltpu.VMEM((DH, F), u32),
            pltpu.VMEM((S, D), f32),
            pltpu.VMEM((TB, 128), f32),
            pltpu.VMEM((L, H * L), f32),
            pltpu.VMEM((H * L // 2, D), u32),
            pltpu.VMEM((L, D), f32),
            pltpu.VMEM((L, HP * 128), f32),
            pltpu.VMEM((HP * 64, D), u32),
            pltpu.VMEM((NB, F // 2, TB), u32),
            pltpu.VMEM((2, D, TB), f32),
            pltpu.VMEM((2, TB, D), f32),
            pltpu.VMEM((4, D, TB), bf16),
            pltpu.SemaphoreType.DMA((4,)),
            pltpu.SemaphoreType.DMA((3,)),
            pltpu.SemaphoreType.DMA((4, HP)),
            pltpu.SemaphoreType.DMA((4,)),
        ],
        compiler_params=pltpu.CompilerParams(vmem_limit_bytes=100 * 1024 * 1024),
    )(A_x.reshape(S, D).T, A_mem0.reshape(M, D), A_Wq, A_Wk, A_Wv,
      A_Wo.transpose(0, 2, 1).reshape(H * D, E), B_w1, B_w2.T)
    return outT.T.reshape(1, S, D)
```

```python
import functools

import jax
import jax.numpy as jnp
from jax import lax
import jax.experimental.pallas as pl
import jax.experimental.pallas.tpu as pltpu

S, D, H, E, F, M, SEG = 2048, 448, 16, 256, 1792, 8, 32
L = M + SEG
HP = H // 2
TB = 128
NB = S // TB
DH = D // 2
DM = 192
NC = F // 128
NA, NM = 4, 10
EPS = 1e-5
SCALE = E ** -0.5
LOG2E = 1.4426950408889634
NSTEPS = S // SEG

T_NT = {t: sorted({(g // 5) // 2 for g in range(16 * t, 16 * t + 16)}) for t in range(5)}
T_LAST = {n: max(t for t in T_NT if n in T_NT[t]) for n in range(HP)}

ORDER = (
    "Q0 Q1 Q2 Q3 Q5 R0 Q4 R1 Q6 S0 Q7 S1 Q8 Q9 R2 Q11 R3 Q10 S2 X0 R4 X1 "
    "T0 S3 Q12 Q13 R5 X2 Q14 Q15 R6 X3 S6 S4 T1 X5 R7 X4 X6 S5 P0:2 S7 X7 F0:48 "
    "T2 F48:80 P2:3 T3 T4 P3:4 U0:4 P4:5 U4:6 U6:8 F80:112 "
).split()

f32, bf16, u32 = jnp.float32, jnp.bfloat16, jnp.uint32
NN = (((1,), (0,)), ((), ()))
NT = (((1,), (1,)), ((), ()))


def _bf(words):
    return pltpu.bitcast(words, bf16)


def _u(vals):
    return pltpu.bitcast(vals, u32)


def _mm(a, b, dims=NN):
    return lax.dot_general(a, b, dims, preferred_element_type=f32)


def _unpack(words, half):
    return pltpu.unpack_elementwise(words, index=half, packed_dtype=bf16, unpacked_dtype=f32)


def _kernel(xT_hbm, mem_hbm, wq_hbm, wk_hbm, wv_hbm, woT_hbm, w1_hbm, w2T_hbm, oT_hbm,
            vw, wraw, obuf, astage, w2T, w1, oacc, wq, wkm, gk, xT, hlast, wb, wtl, xn, tbuf, hidT, membuf, hbuf, woT, pall, sems, xsems, wsems, osems):
    w1_u, woT_u = w1_hbm.bitcast(u32), woT_hbm.bitcast(u32)
    wsrc = [w.bitcast(u32) for w in (wq_hbm, wk_hbm, wv_hbm)]

    def x_copy(i):
        cols = (pl.ds(0, NA * TB), pl.ds(NA * TB, (NM - NA) * TB), pl.ds(NM * TB, S - NM * TB))[i]
        return pltpu.make_async_copy(xT_hbm.at[:, cols], xT.at[:, cols], xsems.at[i])

    def w1_copy(i):
        cols = pl.ds(i * (F // 2), F // 2)
        return pltpu.make_async_copy(w1_u.at[:, cols], w1.at[:, cols], sems.at[1 + 2 * i])

    def w_copy(j, g):
        return pltpu.make_async_copy(wsrc[j].at[:, g, :], wraw.at[j, g], wsems.at[j, g])

    def wo_copy(g):
        rows = pl.ds(pl.multiple_of(g * D, 8), D)
        return pltpu.make_async_copy(woT_u.at[rows, :], woT.at[rows, :], wsems.at[3, g])

    def pair_wait(g):
        wo_copy(g).wait()
        for j in range(3):
            w_copy(j, g).wait()

    mem_copy = pltpu.make_async_copy(mem_hbm, membuf, sems.at[2])
    w2_copy = pltpu.make_async_copy(w2T_hbm.bitcast(u32), w2T, sems.at[0])
    mem_copy.start()
    x_copy(0).start()
    w1_copy(0).start()
    w1_copy(1).start()
    x_copy(1).start()
    x_copy(2).start()
    for g in range(HP):
        wo_copy(g).start()
        for j in (2, 0, 1):
            w_copy(j, g).start()
    w2_copy.start()
    astage[...] = jnp.zeros_like(astage)
    oacc[1] = jnp.zeros_like(oacc[1])

    def ln_block(b):
        xv = xT[:, b * TB:(b + 1) * TB].astype(f32)
        xc = xv - jnp.mean(xv, axis=0, keepdims=True)
        var = jnp.mean(xc * xc, axis=0, keepdims=True)
        xn[b * TB:(b + 1) * TB, :] = (xc * lax.rsqrt(var + EPS)).T

    def ffn1_finish(b, c, h1):
        hv = h1 * pl.reciprocal(1.0 + jnp.exp2(h1 * (-LOG2E)), approx=True)
        hidT[b, c * 64:(c + 1) * 64, :] = _u(hv.T.astype(bf16))

    def ffn1(tiles, items=(), prev=None):
        for n, (b, c) in enumerate(tiles):
            if c == tiles[0][1] or n == 0:
                lhs = xn[pl.ds(pl.multiple_of(b * TB, TB), TB), :]
            h1 = _mm(lhs, _bf(w1[:, c * 128:(c + 1) * 128]))
            if prev is not None:
                ffn1_finish(*prev)
            for item in items[n * len(items) // len(tiles):(n + 1) * len(items) // len(tiles)]:
                item()
            prev = (b, c, h1)
        hlast[...] = prev[2]
        return prev[:2]

    def pair_items(g):
        items = []
        for t in range(2):
            ro = pl.multiple_of((2 * g + t) * DH, 8)
            for m in range(2):

                def retile_qk(t=t, m=m, ro=ro):
                    val = _unpack(wraw[0, g, m * DH:(m + 1) * DH, :], t)
                    wq[pl.ds(ro + m * (DH // 2), DH // 2), :] = _u(val.astype(bf16))
                    val = _unpack(wraw[1, g, m * DH:(m + 1) * DH, :], t)
                    rk = pl.multiple_of((2 * g + t) * DM, 8)
                    if m == 0:
                        wkm[pl.ds(rk, DH // 2), :] = _u(val.astype(bf16))
                    else:
                        nm = 2 * DM - DH
                        wkm[pl.ds(rk + DH // 2, nm // 2), :] = _u(val[:nm].astype(bf16))
                        kt = val[nm:].T
                        parts = [jnp.zeros_like(kt), kt] if t == 0 else [kt, jnp.zeros_like(kt)]
                        gk[pl.ds(pl.multiple_of((2 * g + t) * 128, 8), 128), :] = _u(
                            jnp.concatenate(parts, axis=1).astype(bf16))

                def fold(n, t=t, m=m, ro=ro):
                    wv = _unpack(wraw[2, g, m * DH:(m + 1) * DH, :], t)
                    wo = _bf(woT[pl.ds(ro + n * 64, 64 if n < 3 else 32), :])
                    bu = _u(_mm(wv, wo, NT).astype(bf16))
                    if n < 3:
                        cb, ct = slice(t * 384 + n * 128, t * 384 + (n + 1) * 128), slice(n * 128, (n + 1) * 128)
                    else:
                        cb, ct = slice(768 + t * 64, 768 + (t + 1) * 64), slice(384, D)
                    rb = pl.multiple_of(g * DM, 8)
                    if m == 0:
                        wb[pl.ds(rb, DH // 2), cb] = bu
                    else:
                        nm = DM - DH // 2
                        wb[pl.ds(rb + DH // 2, nm), cb] = bu[:nm]
                        wtl[pl.ds(pl.multiple_of(g * 64, 8) + 32 * t, 32), ct] = bu[nm:]

                items.append(retile_qk)
                items.extend(functools.partial(fold, n) for n in range(4))
        return items

    lo, hi, both = range(NC // 2), range(NC // 2, NC), range(NC)
    x_copy(0).wait()
    for b in range(NA):
        ln_block(b)
    w1_copy(0).wait()
    last = ffn1([(b, c) for b in (0, 1) for c in lo])
    w1_copy(1).wait()
    ffn1_finish(*last, hlast[...])
    last = ffn1([(b, c) for b in (0, 1) for c in hi])
    x_copy(1).wait()
    ffn1_finish(*last, hlast[...])
    last = ffn1([(2, c) for c in both], [functools.partial(ln_block, b) for b in range(NA, NM)])
    x_copy(2).wait()
    ffn1_finish(*last, hlast[...])
    ffn1([(3, c) for c in both], [functools.partial(ln_block, b) for b in range(NM, NB)])

    def prologue_body(i, carry):
        pair_wait(i - 2)
        ffn1([(2 * i + t, c) for t in range(2) for c in both], pair_items(i - 2),
             prev=(2 * i - 1, NC - 1, hlast[...]))
        return carry

    lax.fori_loop(2, NB // 2, prologue_body, 0)
    pair_wait(HP - 2)
    pair_wait(HP - 1)
    ffn1_finish(NB - 1, NC - 1, hlast[...])
    for item in pair_items(HP - 2) + pair_items(HP - 1):
        item()
    w2_copy.wait()
    mem_copy.wait()

    row = lax.broadcasted_iota(jnp.int32, (L, 128), 0)
    lane = lax.broadcasted_iota(jnp.int32, (L, 128), 1)
    low = lane < 64
    col = lane % 64
    mask2 = (col < L) & ((row < M) | (row >= col))

    def step(b, slot, j, mem):
        hbuf[0:M, :] = mem
        hbuf[M:L, :] = xn[pl.ds(pl.multiple_of(b * TB + j * SEG, SEG), SEG), :]
        ht = hbuf[:, 2 * DM:D]
        ht_lane = (jnp.concatenate([ht, jnp.zeros_like(ht)], axis=1),
                   jnp.concatenate([jnp.zeros_like(ht), ht], axis=1))
        zero8 = jnp.zeros((8, 128), f32)
        qk, part, tacc, acc = {}, {}, {}, []

        def keys_t(blk, odd):
            if not odd:
                return jnp.pad(blk.T, ((0, 0), (0, 128 - L)))
            return jnp.concatenate([jnp.zeros((64, 128), f32), blk, jnp.zeros((64 - L, 128), f32)], axis=0).T

        zmat = jnp.concatenate([keys_t(ht_lane[0], True)[:64], keys_t(ht_lane[0], False)[:64]], axis=0).astype(bf16)

        def qk_proj(h):
            q = _mm(hbuf[...], _bf(wq[h * DH:(h + 1) * DH, :]))
            km = _mm(hbuf[:, 0:2 * DM], _bf(wkm[h * DM:(h + 1) * DM, :]))
            kt = jnp.concatenate([keys_t(km[:, c * 128:(c + 1) * 128], h % 2) for c in range(2)], axis=0)
            qk[h] = (q, _bf(_u(kt.astype(bf16)) | gk[h * 128:(h + 1) * 128, :]))

        def scores(g):
            oa = _mm(*qk[2 * g])
            ob = _mm(*qk[2 * g + 1])
            part[g] = (jnp.where(low, oa, ob), jnp.where(low, ob, oa))

        def softmax(g):
            sm, v1 = part[g]
            sc = jnp.where(mask2, (sm + _mm(v1, zmat)) * SCALE, -1e9)
            mx = jnp.where(low, jnp.max(jnp.where(low, sc, -1e9), axis=-1, keepdims=True),
                           jnp.max(jnp.where(low, -1e9, sc), axis=-1, keepdims=True))
            p = jnp.exp(sc - mx)
            sa = jnp.sum(jnp.where(low, p, 0.0), axis=-1, keepdims=True)
            sb = jnp.sum(jnp.where(low, 0.0, p), axis=-1, keepdims=True)
            p = p * pl.reciprocal(jnp.where(low, sa, sb), approx=True)
            pall[:, 2 * g * L:(2 * g + 1) * L] = p[:, 0:L]
            pall[:, (2 * g + 1) * L:(2 * g + 2) * L] = p[:, 64:64 + L]

        def value_main(g):
            hb = _mm(hbuf[:, 0:2 * DM], _bf(wb[g * DM:(g + 1) * DM, :]))
            va = jnp.concatenate([hb[:, 0:384], hb[:, 768:832]], axis=1)
            vb = jnp.concatenate([hb[:, 384:768], hb[:, 832:896]], axis=1)
            vw[g * L:(g + 1) * L, :] = _u(jnp.concatenate([va, vb], axis=0).astype(bf16))

        def t_tile(t):
            cols = []
            for n in T_NT[t]:
                rows = []
                for g in range(16 * t, 16 * t + 16):
                    h, k = g // 5, g % 5
                    rows.append(ht_lane[h % 2][8 * k:8 * k + 8] if h // 2 == n else zero8)
                cols.append(jnp.concatenate(rows, axis=0))
            r = _mm(pall[:, t * 128:(t + 1) * 128], jnp.concatenate(cols, axis=1).astype(bf16))
            for i, n in enumerate(T_NT[t]):
                part = r[:, i * 128:(i + 1) * 128]
                tacc[n] = tacc[n] + part if n in tacc else part
                if T_LAST[n] == t:
                    tbuf[:, n * 128:(n + 1) * 128] = tacc[n]

        def accumulate(r):
            acc[:] = [acc[0] + r if acc else r]

        def p_tiles(t0, t1):
            accumulate(_mm(pall[:, t0 * 128:t1 * 128], _bf(vw[t0 * 64:t1 * 64, :])))

        def u_tiles(g0, g1):
            accumulate(_mm(tbuf[:, g0 * 128:g1 * 128], _bf(wtl[g0 * 64:g1 * 64, :])))

        def ffn2(r0, r1):
            w = _bf(w2T[pl.ds((j * (D // 4) + r0) // 2, (r1 - r0) // 2), :])
            oacc[slot, pl.ds(j * (D // 4) + r0, r1 - r0), :] = _mm(w, _bf(hidT[b]))

        ops = dict(Q=qk_proj, R=scores, S=softmax, X=value_main, T=t_tile, P=p_tiles, U=u_tiles, F=ffn2)
        for op in ORDER:
            ops[op[0]](*(int(v) for v in op[1:].split(":")))
        out = acc[0]
        astage[slot, pl.ds(j * SEG, SEG), :] = out[M:, :]
        return out[:M, :]

    def finish_block(b, slot, oslot):
        xb = xT[:, pl.ds(pl.multiple_of(b * TB, TB), TB)].astype(f32)
        obuf[oslot] = (xb + oacc[slot] + astage[slot].T).astype(bf16)

    def out_copy(b):
        cols = pl.ds(pl.multiple_of(b * TB, TB), TB)
        return pltpu.make_async_copy(obuf.at[b % 4], oT_hbm.at[:, cols], osems.at[b % 4])

    def two_blocks(i, mem):
        b = 2 * i

        @pl.when(i >= 2)
        def _():
            out_copy(b - 4).wait()

        @pl.when(i >= 3)
        def _():
            out_copy(b - 5).wait()

        finish_block(jnp.maximum(b - 1, 0), 1, (b + 3) % 4)
        for j in range(4):
            mem = step(b, 0, j, mem)
        finish_block(b, 0, b % 4)
        for j in range(4):
            mem = step(b + 1, 1, j, mem)

        @pl.when(i >= 1)
        def _():
            out_copy(b - 1).start()

        out_copy(b).start()
        return mem

    lax.fori_loop(0, NSTEPS // 8, two_blocks, membuf[...].astype(f32))

    nb = NSTEPS // 4
    out_copy(nb - 5).wait()
    finish_block(nb - 1, 1, (nb - 1) % 4)
    out_copy(nb - 1).start()
    for b in range(nb - 4, nb):
        out_copy(b).wait()


@jax.jit
def pallas_parallel_sum__memory_aug_recurrent_mem_tr__dense_activation_silu__prompt_kernel(A_x, A_mem0, A_Wq, A_Wk, A_Wv, A_Wo, A_seg_len, B_x, B_w1, B_w2):
    del A_seg_len, B_x
    hbm = pl.BlockSpec(memory_space=pltpu.HBM)
    outT = pl.pallas_call(
        _kernel,
        out_shape=jax.ShapeDtypeStruct((D, S), A_x.dtype),
        in_specs=[hbm] * 8,
        out_specs=hbm,
        scratch_shapes=[
            pltpu.VMEM((H * L // 2, D), u32),
            pltpu.VMEM((3, HP, D, E), u32),
            pltpu.VMEM((4, D, TB), bf16),
            pltpu.VMEM((2, TB, D), f32),
            pltpu.VMEM((DH, F), u32),
            pltpu.VMEM((DH, F), u32),
            pltpu.VMEM((2, D, TB), f32),
            pltpu.VMEM((H * DH, E), u32),
            pltpu.VMEM((H * DM, E), u32),
            pltpu.VMEM((H * 128, 128), u32),
            pltpu.VMEM((D, S), bf16),
            pltpu.VMEM((TB, 128), f32),
            pltpu.VMEM((HP * DM, 2 * D), u32),
            pltpu.VMEM((HP * 64, D), u32),
            pltpu.VMEM((S, D), f32),
            pltpu.VMEM((L, HP * 128), f32),
            pltpu.VMEM((NB, F // 2, TB), u32),
            pltpu.VMEM((M, D), bf16),
            pltpu.VMEM((L, D), f32),
            pltpu.VMEM((H * DH, E), u32),
            pltpu.VMEM((L, H * L), f32),
            pltpu.SemaphoreType.DMA((4,)),
            pltpu.SemaphoreType.DMA((3,)),
            pltpu.SemaphoreType.DMA((4, HP)),
            pltpu.SemaphoreType.DMA((4,)),
        ],
        compiler_params=pltpu.CompilerParams(vmem_limit_bytes=100 * 1024 * 1024),
    )(A_x.reshape(S, D).T, A_mem0.reshape(M, D), A_Wq, A_Wk, A_Wv,
      A_Wo.transpose(0, 2, 1).reshape(H * D, E), B_w1, B_w2.T)
    return outT.T.reshape(1, S, D)
```
